```python
import jax
import jax.numpy as jnp

def _softmax(x, axis=-1):
    return jax.nn.softmax(x, axis=axis)

def _gelu(x):
    return jax.nn.gelu(x, approximate=True)

def _silu(x):
    return jax.nn.silu(x)

def _sigmoid(x):
    return jax.nn.sigmoid(x)

def _layernorm(x, axis=-1, eps=1e-05):
    m = jnp.mean(x, axis=axis, keepdims=True)
    v = jnp.var(x, axis=axis, keepdims=True)
    return (x - m) / jnp.sqrt(v + eps)

def _scatter_add(tgt, idx, src, axis=0):
    return tgt.at[idx].add(src)

def _segment_sum(src, seg, n):
    return jax.ops.segment_sum(src, seg, n)

class _Rng:

    def __init__(self, key):
        self._k = key

    def _next(self):
        self._k, sub = jax.random.split(self._k)
        return sub

    def normal(self, shape):
        return jax.random.normal(self._next(), shape, dtype=jnp.bfloat16)

    def randint(self, lo, hi, shape):
        return jax.random.randint(self._next(), shape, lo, hi, dtype=jnp.int32)

    def uniform(self, shape, lo=0.0, hi=1.0):
        return jax.random.uniform(self._next(), shape, jnp.bfloat16, lo, hi)

    def permutation(self, n):
        return jax.random.permutation(self._next(), n)
kernel_name = 'interleave_layers__linear_kernel_hedgehog__memory_aug_recurrent_mem_tr__prompt'

def setup_inputs():
    _rng = _Rng(jax.random.key(int.from_bytes(__import__("os").urandom(4), "little")))
    _w = lambda a: (lambda t: t.astype(jnp.bfloat16) if jnp.issubdtype(t.dtype, jnp.floating) else t)(jnp.asarray(a))

    def _A_setup():
        B, S, D, H = (1, 2048, 640, 32)
        Dh = D // H
        return {'x': _w((lambda *s: _rng.normal(s) * 0.05)(B, S, D)), 'wqkv': _w((lambda *s: _rng.normal(s) * 0.05)(D, 3 * D)), 'w_phi': _w((lambda *s: _rng.normal(s) * 0.05)(H, Dh, Dh) * Dh ** (-0.5)), 'wo': _w((lambda *s: _rng.normal(s) * 0.05)(D, D))}
    _A_in = _A_setup()

    def _B_setup():
        B, S, Dm = (1, 2048, 640)
        H, Dh = (32, 192)
        M, seg = (8, 32)
        seg = min(seg, S)
        S = S // seg * seg
        return {'x': _w((lambda *s: _rng.normal(s) * 0.05)(B, S, Dm)), 'mem0': _w((lambda *s: _rng.normal(s) * 0.05)(B, M, Dm)), 'Wq': _w((lambda *s: _rng.normal(s) * 0.05)(Dm, H, Dh) * Dm ** (-0.5)), 'Wk': _w((lambda *s: _rng.normal(s) * 0.05)(Dm, H, Dh) * Dm ** (-0.5)), 'Wv': _w((lambda *s: _rng.normal(s) * 0.05)(Dm, H, Dh) * Dm ** (-0.5)), 'Wo': _w((lambda *s: _rng.normal(s) * 0.05)(H, Dh, Dm) * (H * Dh) ** (-0.5)), 'seg_len': seg}
    _B_in = _B_setup()
    return {'A_x': _A_in['x'], 'A_wqkv': _A_in['wqkv'], 'A_w_phi': _A_in['w_phi'], 'A_wo': _A_in['wo'], 'B_x': _B_in['x'], 'B_mem0': _B_in['mem0'], 'B_Wq': _B_in['Wq'], 'B_Wk': _B_in['Wk'], 'B_Wv': _B_in['Wv'], 'B_Wo': _B_in['Wo'], 'B_seg_len': _B_in['seg_len']}

def reference(A_x, A_wqkv, A_w_phi, A_wo, B_x, B_mem0, B_Wq, B_Wk, B_Wv, B_Wo, B_seg_len):

    def _A_ref(x, wqkv, w_phi, wo):
        B, S, D = x.shape
        H = 32
        Dh = D // H
        qkv = (lambda x, *d: x.transpose(*d))((x @ wqkv).reshape(B, S, 3, H, Dh), 2, 0, 3, 1, 4)
        q, k, v = (qkv[0], qkv[1], qkv[2])
        pq = jnp.einsum('bhsd,hdf->bhsf', q, w_phi)
        pk = jnp.einsum('bhsd,hdf->bhsf', k, w_phi)
        phi_q = jnp.concatenate([_softmax(pq, axis=-1), _softmax(-pq, axis=-1)], axis=-1)
        phi_k = jnp.concatenate([_softmax(pk, axis=-1), _softmax(-pk, axis=-1)], axis=-1)
        kv = jnp.einsum('bhsf,bhsd->bhfd', phi_k, v)
        z = jnp.einsum('bhsf->bhf', phi_k)
        num = jnp.einsum('bhqf,bhfd->bhqd', phi_q, kv)
        den = jnp.einsum('bhqf,bhf->bhq', phi_q, z)[..., None] + 1e-06
        o = num / den
        return (lambda x, *d: x.transpose(*d))(o, 0, 2, 1, 3).reshape(B, S, D) @ wo

    def _B_ref(x, mem0, Wq, Wk, Wv, Wo, seg_len):
        B, S, Dm = x.shape
        H, Dh = (Wq.shape[1], Wq.shape[2])
        M = mem0.shape[1]
        scale = Dh ** (-0.5)
        n_seg = S // seg_len
        L = M + seg_len
        idx = jnp.arange(L)
        mask = (idx[:, None] < M) | (idx[:, None] >= idx[None, :])
        mem = mem0
        outs = []
        for s in range(n_seg):
            xs = x[:, s * seg_len:(s + 1) * seg_len, :].copy()
            h = jnp.concatenate([mem, xs], axis=1)
            q = jnp.einsum('btd,dhe->bhte', h, Wq)
            k = jnp.einsum('btd,dhe->bhte', h, Wk)
            v = jnp.einsum('btd,dhe->bhte', h, Wv)
            scores = jnp.einsum('bhqe,bhke->bhqk', q, k) * scale
            scores = jnp.where(mask[None, None], scores, -1000000000.0)
            p = _softmax(scores, axis=-1)
            o = jnp.einsum('bhqk,bhke->bhqe', p, v)
            o = jnp.einsum('bhte,hed->btd', o, Wo)
            mem = o[:, :M, :].copy()
            outs.append(o[:, M:, :])
        return jnp.concatenate(outs, axis=1)
    x = A_x
    x = x + _A_ref(_layernorm(x, axis=-1), A_wqkv, A_w_phi, A_wo)
    x = x + _B_ref(_layernorm(x, axis=-1), B_mem0, B_Wq, B_Wk, B_Wv, B_Wo, B_seg_len)
    x = x + _A_ref(_layernorm(x, axis=-1), A_wqkv, A_w_phi, A_wo)
    x = x + _B_ref(_layernorm(x, axis=-1), B_mem0, B_Wq, B_Wk, B_Wv, B_Wo, B_seg_len)
    return x
```

```python
import functools
import jax
import jax.numpy as jnp
from jax import lax
import jax.experimental.pallas as pl
import jax.experimental.pallas.tpu as pltpu

F32, BF = jnp.float32, jnp.bfloat16
HA = 32
CH = 256


def _dot(a, b):
    return jnp.dot(a, b, preferred_element_type=F32)


def _dg(a, b, ca, cb):
    return lax.dot_general(a, b, (((ca,), (cb,)), ((), ())), preferred_element_type=F32)


def _ln(x):
    m = jnp.mean(x, axis=-1, keepdims=True)
    d = x - m
    v = jnp.mean(d * d, axis=-1, keepdims=True)
    return d * lax.rsqrt(v + 1e-5)


def _iota(shape, ax):
    return lax.broadcasted_iota(jnp.int32, shape, ax)


def _tiles(a):
    return [a[:, i * 128:(i + 1) * 128] for i in range(a.shape[1] // 128)]


def _allred(ts, op):
    r = functools.reduce(op, ts)
    r = op(r, pltpu.roll(r, 64, 1))
    return op(r, pltpu.roll(r, 32, 1))


def _phi(p):
    ts = _tiles(p)
    mx = _allred(ts, jnp.maximum)
    mn = _allred(ts, jnp.minimum)
    out = []
    for e in ([jnp.exp(t - mx) for t in ts], [jnp.exp(mn - t) for t in ts]):
        inv = 1.0 / _allred(e, jnp.add)
        out += [t * inv for t in e]
    return out


def _kernel(seg, x_ref, wqkv_ref, wphi_ref, wo_ref, mem_ref, wq_h, wk_h, wv_h, wob_h,
            o_ref, xs, wqk, phiq, wq, wk, wv, wob, sem):
    S, D = xs.shape
    M = mem_ref.shape[0]
    dh = D // HA
    L = M + seg
    E = 192
    cps = [pltpu.make_async_copy(s, d, sem.at[i]) for i, (s, d) in
           enumerate(((wq_h, wq), (wk_h, wk), (wv_h, wv), (wob_h, wob)))]
    for c in cps:
        c.start()

    rep = (_iota((dh, D), 0) == _iota((dh, D), 1) // HA).astype(BF)
    bd = _dot(wphi_ref[...], rep)
    bd = jnp.where(_iota((D, D), 0) // dh == _iota((D, D), 1) % HA, bd, 0.0).astype(BF)
    wqk[:, :D] = _dot(wqkv_ref[:, :D], bd).astype(BF)
    wqk[:, D:] = _dot(wqkv_ref[:, D:2 * D], bd).astype(BF)
    xs[...] = x_ref[...].astype(F32)

    def layer_a():
        def p1(i, c):
            kvt, z = c
            r = pl.ds(pl.multiple_of(i * CH, CH), CH)
            h = _ln(xs[r, :]).astype(BF)
            phiq[r, :] = jnp.concatenate(_phi(_dot(h, wqk[:, :D])), axis=1).astype(BF)
            pk = jnp.concatenate(_phi(_dot(h, wqk[:, D:])), axis=1)
            v = _dot(h, wqkv_ref[:, 2 * D:]).astype(BF)
            return kvt + _dg(v, pk.astype(BF), 0, 0), z + jnp.sum(pk, axis=0, keepdims=True)

        kvt, z = lax.fori_loop(0, S // CH, p1, (jnp.zeros((D, 2 * D), F32), jnp.zeros((1, 2 * D), F32)))
        kvt = jnp.where(_iota((D, 2 * D), 0) // dh == _iota((D, 2 * D), 1) % HA, kvt, 0.0).astype(BF)
        g = _dg(kvt, wo_ref[...], 0, 0).astype(BF)

        def p2(i, c):
            r = pl.ds(pl.multiple_of(i * CH, CH), CH)
            ts = _tiles(phiq[r, :].astype(F32))
            inv = 1.0 / (_allred([t * zt for t, zt in zip(ts, _tiles(z))], jnp.add) + 1e-6)
            xs[r, :] += _dot(jnp.concatenate([t * inv for t in ts], axis=1).astype(BF), g)
            return c

        lax.fori_loop(0, S // CH, p2, 0)

    def layer_b():
        scale = E ** -0.5
        qi = _iota((2 * L, L), 0) % L
        mask = (qi < M) | (qi >= _iota((2 * L, L), 1))
        lo = _iota((L, 128), 1) < 64

        def step(s, mem):
            r = pl.ds(pl.multiple_of(s * seg, seg), seg)
            xr = xs[r, :]
            h = jnp.concatenate([mem, _ln(xr)], axis=0).astype(BF)
            acc = jnp.zeros((L, D), F32)
            for p in range(wq.shape[1] // (2 * E)):
                c = slice(p * 2 * E, (p + 1) * 2 * E)
                q0, q1, q2 = _tiles(_dot(h, wq[:, c]))
                k0, k1, k2 = _tiles(_dot(h, wk[:, c]).astype(BF))
                v0, v1, v2 = _tiles(_dot(h, wv[:, c]).astype(BF))
                qm = jnp.concatenate([jnp.where(lo, q1, 0.0), jnp.where(lo, 0.0, q1)], axis=0)
                sc = _dg(qm.astype(BF), k1, 1, 1) + jnp.concatenate(
                    [_dg(q0.astype(BF), k0, 1, 1), _dg(q2.astype(BF), k2, 1, 1)], axis=0)
                sc = jnp.where(mask, sc * scale, -1e9)
                e = jnp.exp(sc - jnp.max(sc, axis=-1, keepdims=True))
                pr = e * (1.0 / jnp.sum(e, axis=-1, keepdims=True))
                om = _dot(pr.astype(BF), v1)
                o = jnp.concatenate([_dot(pr[:L].astype(BF), v0), jnp.where(lo, om[:L], om[L:]),
                                     _dot(pr[L:].astype(BF), v2)], axis=1)
                acc = acc + _dot(o.astype(BF), wob[c, :])
            xs[r, :] = xr + acc[M:]
            return acc[:M]

        lax.fori_loop(0, S // seg, step, mem_ref[...].astype(F32))

    def layers(i, c):
        layer_a()

        @pl.when(i == 0)
        def _():
            for cp in cps:
                cp.wait()

        layer_b()
        return c

    lax.fori_loop(0, 2, layers, 0)
    o_ref[...] = xs[...].astype(o_ref.dtype)


def pallas_interleave_layers__linear_kernel_hedgehog__memory_aug_recurrent_mem_tr__prompt_kernel(
        A_x, A_wqkv, A_w_phi, A_wo, B_x, B_mem0, B_Wq, B_Wk, B_Wv, B_Wo, B_seg_len=32):
    _, S, D = A_x.shape
    seg = B_seg_len if isinstance(B_seg_len, int) else 32
    HE = B_Wq.shape[1] * B_Wq.shape[2]
    vm = pl.BlockSpec(memory_space=pltpu.VMEM)
    hb = pl.BlockSpec(memory_space=pl.ANY)
    out = pl.pallas_call(
        functools.partial(_kernel, seg),
        in_specs=[vm] * 5 + [hb] * 4,
        out_specs=vm,
        out_shape=jax.ShapeDtypeStruct((S, D), A_x.dtype),
        scratch_shapes=[pltpu.VMEM((S, D), F32), pltpu.VMEM((D, 2 * D), BF), pltpu.VMEM((S, 2 * D), BF),
                        pltpu.VMEM((D, HE), BF), pltpu.VMEM((D, HE), BF), pltpu.VMEM((D, HE), BF),
                        pltpu.VMEM((HE, D), BF), pltpu.SemaphoreType.DMA((4,))],
        compiler_params=pltpu.CompilerParams(vmem_limit_bytes=110 * 1024 * 1024),
    )(A_x.reshape(S, D), A_wqkv, A_w_phi.reshape(D, D // HA), A_wo, B_mem0.reshape(-1, D),
      B_Wq.reshape(D, HE), B_Wk.reshape(D, HE), B_Wv.reshape(D, HE), B_Wo.reshape(HE, D))
    return out.reshape(1, S, D)
```

```python
import functools
import jax
import jax.numpy as jnp
from jax import lax
import jax.experimental.pallas as pl
import jax.experimental.pallas.tpu as pltpu

F32, BF = jnp.float32, jnp.bfloat16
HA = 32
G = 16
CH = 256


def _dot(a, b):
    return jnp.dot(a, b, preferred_element_type=F32)


def _dg(a, b, ca, cb):
    return lax.dot_general(a, b, (((ca,), (cb,)), ((), ())), preferred_element_type=F32)


def _ln(x):
    m = jnp.mean(x, axis=-1, keepdims=True)
    d = x - m
    v = jnp.mean(d * d, axis=-1, keepdims=True)
    return d * lax.rsqrt(v + 1e-5)


def _iota(shape, ax):
    return lax.broadcasted_iota(jnp.int32, shape, ax)


def _tiles(a):
    return [a[:, i * 128:(i + 1) * 128] for i in range(a.shape[1] // 128)]


def _allred(ts, op):
    r = functools.reduce(op, ts)
    r = op(r, pltpu.roll(r, 64, 1))
    return op(r, pltpu.roll(r, 32, 1))


def _phi(p):
    ts = _tiles(p)
    mx = _allred(ts, jnp.maximum)
    mn = _allred(ts, jnp.minimum)
    out = []
    for e in ([jnp.exp(t - mx) for t in ts], [jnp.exp(mn - t) for t in ts]):
        inv = 1.0 / _allred(e, jnp.add)
        out += [t * inv for t in e]
    return out


def _kernel(seg, x_ref, wqkv_ref, wphi_ref, wo_ref, mem_ref, wq_h, wk_h, wv_h, wob_h,
            o_ref, xs, wqk, phiq, wq, wk, wv, wob, sem):
    S, D = xs.shape
    M = mem_ref.shape[0]
    dh = D // HA
    L = seg + 2 * M
    E = 192
    cps = [pltpu.make_async_copy(s, d, sem.at[i]) for i, (s, d) in
           enumerate(((wq_h, wq), (wk_h, wk), (wv_h, wv), (wob_h, wob)))]
    for c in cps:
        c.start()

    rep = (_iota((dh, D), 0) == _iota((dh, D), 1) // HA).astype(BF)
    bd = _dot(wphi_ref[...], rep)
    bd = jnp.where(_iota((D, D), 0) // dh == _iota((D, D), 1) % HA, bd, 0.0).astype(BF)
    wqk[:, :D] = _dot(wqkv_ref[:, :D], bd).astype(BF)
    wqk[:, D:] = _dot(wqkv_ref[:, D:2 * D], bd).astype(BF)
    xs[...] = x_ref[...].astype(F32)

    def layer_a():
        def p1(i, c):
            kvt, z = c
            r = pl.ds(pl.multiple_of(i * CH, CH), CH)
            h = _ln(xs[r, :]).astype(BF)
            phiq[r, :] = jnp.concatenate(_phi(_dot(h, wqk[:, :D])), axis=1).astype(BF)
            pk = jnp.concatenate(_phi(_dot(h, wqk[:, D:])), axis=1)
            v = _dot(h, wqkv_ref[:, 2 * D:]).astype(BF)
            return kvt + _dg(v, pk.astype(BF), 0, 0), z + jnp.sum(pk, axis=0, keepdims=True)

        kvt, z = lax.fori_loop(0, S // CH, p1, (jnp.zeros((D, 2 * D), F32), jnp.zeros((1, 2 * D), F32)))
        kvt = jnp.where(_iota((D, 2 * D), 0) // dh == _iota((D, 2 * D), 1) % HA, kvt, 0.0).astype(BF)
        g = _dg(kvt, wo_ref[...], 0, 0).astype(BF)

        def p2(i, c):
            r = pl.ds(pl.multiple_of(i * CH, CH), CH)
            ts = _tiles(phiq[r, :].astype(F32))
            inv = 1.0 / (_allred([t * zt for t, zt in zip(ts, _tiles(z))], jnp.add) + 1e-6)
            xs[r, :] += _dot(jnp.concatenate([t * inv for t in ts], axis=1).astype(BF), g)
            return c

        lax.fori_loop(0, S // CH, p2, 0)

    def layer_b():
        scale = E ** -0.5
        qi = _iota((2 * L, L), 0) % L
        ki = _iota((2 * L, L), 1)
        mask = (ki < seg + M) & ((qi >= seg) | (ki >= seg) | (qi >= ki))
        lo = _iota((L, 128), 1) < 64

        def step(s, mem):
            r = pl.ds(pl.multiple_of(s * seg, seg), seg)
            xr = xs[r, :]
            h = jnp.concatenate([_ln(xr), mem, jnp.zeros_like(mem)], axis=0).astype(BF)
            W = G * 2 * E
            ng = wq.shape[1] // W

            def proj(g):
                c = slice(g * W, (g + 1) * W)
                return (_tiles(_dot(h, wq[:, c])), _tiles(_dot(h, wk[:, c]).astype(BF)),
                        _tiles(_dot(h, wv[:, c]).astype(BF)))

            def qk(q, k):
                q0, q1, q2 = q
                k0, k1, k2 = k
                qm = jnp.concatenate([jnp.where(lo, q1, 0.0), jnp.where(lo, 0.0, q1)], axis=0)
                sc = _dg(qm.astype(BF), k1, 1, 1) + jnp.concatenate(
                    [_dg(q0.astype(BF), k0, 1, 1), _dg(q2.astype(BF), k2, 1, 1)], axis=0)
                return sc

            def sm(sc):
                sc = jnp.where(mask, sc * scale, -1e9)
                e = jnp.exp(sc - jnp.max(sc, axis=-1, keepdims=True))
                pr = e * (1.0 / jnp.sum(e, axis=-1, keepdims=True))
                return pr

            def pv(pr, v):
                v0, v1, v2 = v
                om = _dot(pr.astype(BF), v1)
                o = jnp.concatenate([_dot(pr[:L].astype(BF), v0), jnp.where(lo, om[:L], om[L:]),
                                     _dot(pr[L:].astype(BF), v2)], axis=1)
                return o.astype(BF)

            acc = None
            cur = proj(0)
            for g in range(ng):
                nxt = proj(g + 1) if g + 1 < ng else None
                scs = [qk(cur[0][3 * j:3 * j + 3], cur[1][3 * j:3 * j + 3]) for j in range(G)]
                prs = [sm(t) for t in scs]
                o = jnp.concatenate([pv(prs[j], cur[2][3 * j:3 * j + 3]) for j in range(G)], axis=1)
                d = _dot(o, wob[g * W:(g + 1) * W, :])
                acc = d if acc is None else acc + d
                cur = nxt
            xs[r, :] = xr + acc[:seg]
            return acc[seg:seg + M]

        lax.fori_loop(0, S // seg, step, mem_ref[...].astype(F32))

    def layers(i, c):
        layer_a()

        @pl.when(i == 0)
        def _():
            for cp in cps:
                cp.wait()

        layer_b()
        return c

    lax.fori_loop(0, 2, layers, 0)
    o_ref[...] = xs[...].astype(o_ref.dtype)


def pallas_interleave_layers__linear_kernel_hedgehog__memory_aug_recurrent_mem_tr__prompt_kernel(
        A_x, A_wqkv, A_w_phi, A_wo, B_x, B_mem0, B_Wq, B_Wk, B_Wv, B_Wo, B_seg_len=32):
    _, S, D = A_x.shape
    seg = B_seg_len if isinstance(B_seg_len, int) else 32
    HE = B_Wq.shape[1] * B_Wq.shape[2]
    vm = pl.BlockSpec(memory_space=pltpu.VMEM)
    hb = pl.BlockSpec(memory_space=pl.ANY)
    out = pl.pallas_call(
        functools.partial(_kernel, seg),
        in_specs=[vm] * 5 + [hb] * 4,
        out_specs=vm,
        out_shape=jax.ShapeDtypeStruct((S, D), A_x.dtype),
        scratch_shapes=[pltpu.VMEM((S, D), F32), pltpu.VMEM((D, 2 * D), BF), pltpu.VMEM((S, 2 * D), BF),
                        pltpu.VMEM((D, HE), BF), pltpu.VMEM((D, HE), BF), pltpu.VMEM((D, HE), BF),
                        pltpu.VMEM((HE, D), BF), pltpu.SemaphoreType.DMA((4,))],
        compiler_params=pltpu.CompilerParams(vmem_limit_bytes=110 * 1024 * 1024),
    )(A_x.reshape(S, D), A_wqkv, A_w_phi.reshape(D, D // HA), A_wo, B_mem0.reshape(-1, D),
      B_Wq.reshape(D, HE), B_Wk.reshape(D, HE), B_Wv.reshape(D, HE), B_Wo.reshape(HE, D))
    return out.reshape(1, S, D)
```

```python
import functools
import jax
import jax.numpy as jnp
from jax import lax
import jax.experimental.pallas as pl
import jax.experimental.pallas.tpu as pltpu

F32, BF = jnp.float32, jnp.bfloat16
HA = 32
G = 16
CH = 512


def _dot(a, b):
    return jnp.dot(a, b, preferred_element_type=F32)


def _dg(a, b, ca, cb):
    return lax.dot_general(a, b, (((ca,), (cb,)), ((), ())), preferred_element_type=F32)


def _ln(x):
    m = jnp.mean(x, axis=-1, keepdims=True)
    d = x - m
    v = jnp.mean(d * d, axis=-1, keepdims=True)
    return d * lax.rsqrt(v + 1e-5)


def _iota(shape, ax):
    return lax.broadcasted_iota(jnp.int32, shape, ax)


def _tiles(a):
    return [a[:, i * 128:(i + 1) * 128] for i in range(a.shape[1] // 128)]


def _allred(ts, op):
    r = functools.reduce(op, ts)
    r = op(r, pltpu.roll(r, 64, 1))
    return op(r, pltpu.roll(r, 32, 1))


def _phi(p):
    ts = _tiles(p)
    mx = _allred(ts, jnp.maximum)
    mn = _allred(ts, jnp.minimum)
    out = []
    for e in ([jnp.exp(t - mx) for t in ts], [jnp.exp(mn - t) for t in ts]):
        inv = 1.0 / _allred(e, jnp.add)
        out += [t * inv for t in e]
    return out


def _kernel(seg, x_ref, wqkv_ref, wphi_ref, wo_ref, mem_ref, wq_h, wk_h, wv_h, wob_h,
            o_ref, xs, wqk, phiq, wq, wk, wv, wob, sem):
    S, D = xs.shape
    M = mem_ref.shape[0]
    dh = D // HA
    L = seg + 2 * M
    E = 192
    cps = [pltpu.make_async_copy(s, d, sem.at[i]) for i, (s, d) in
           enumerate(((wq_h, wq), (wk_h, wk), (wv_h, wv), (wob_h, wob)))]
    for c in cps:
        c.start()

    rep = (_iota((dh, D), 0) == _iota((dh, D), 1) // HA).astype(BF)
    bd = _dot(wphi_ref[...], rep)
    bd = jnp.where(_iota((D, D), 0) // dh == _iota((D, D), 1) % HA, bd, 0.0).astype(BF)
    wqk[:, :D] = _dot(wqkv_ref[:, :D], bd).astype(BF)
    wqk[:, D:] = _dot(wqkv_ref[:, D:2 * D], bd).astype(BF)
    xs[...] = x_ref[...].astype(F32)

    def layer_a():
        def p1(i, c):
            kvt, z = c
            r = pl.ds(pl.multiple_of(i * CH, CH), CH)
            h = _ln(xs[r, :]).astype(BF)
            phiq[r, :] = jnp.concatenate(_phi(_dot(h, wqk[:, :D])), axis=1).astype(BF)
            pk = jnp.concatenate(_phi(_dot(h, wqk[:, D:])), axis=1)
            v = _dot(h, wqkv_ref[:, 2 * D:]).astype(BF)
            return kvt + _dg(v, pk.astype(BF), 0, 0), z + jnp.sum(pk, axis=0, keepdims=True)

        kvt, z = lax.fori_loop(0, S // CH, p1, (jnp.zeros((D, 2 * D), F32), jnp.zeros((1, 2 * D), F32)))
        kvt = jnp.where(_iota((D, 2 * D), 0) // dh == _iota((D, 2 * D), 1) % HA, kvt, 0.0).astype(BF)
        g = _dg(kvt, wo_ref[...], 0, 0).astype(BF)

        def p2(i, c):
            r = pl.ds(pl.multiple_of(i * CH, CH), CH)
            ts = _tiles(phiq[r, :].astype(F32))
            inv = 1.0 / (_allred([t * zt for t, zt in zip(ts, _tiles(z))], jnp.add) + 1e-6)
            xs[r, :] += _dot(jnp.concatenate([t * inv for t in ts], axis=1).astype(BF), g)
            return c

        lax.fori_loop(0, S // CH, p2, 0)

    def layer_b():
        scale = E ** -0.5
        qi = _iota((2 * L, L), 0) % L
        ki = _iota((2 * L, L), 1)
        mask = (ki < seg + M) & ((qi >= seg) | (ki >= seg) | (qi >= ki))
        lo = _iota((L, 128), 1) < 64

        def step(s, mem):
            r = pl.ds(pl.multiple_of(s * seg, seg), seg)
            xr = xs[r, :]
            h = jnp.concatenate([_ln(xr), mem, jnp.zeros_like(mem)], axis=0).astype(BF)
            W = G * 2 * E
            ng = wq.shape[1] // W

            def proj(g):
                c = slice(g * W, (g + 1) * W)
                return (_tiles(_dot(h, wq[:, c])), _tiles(_dot(h, wk[:, c]).astype(BF)),
                        None)

            def qk(q, k):
                q0, q1, q2 = q
                k0, k1, k2 = k
                qm = jnp.concatenate([jnp.where(lo, q1, 0.0), jnp.where(lo, 0.0, q1)], axis=0)
                sc = _dg(qm.astype(BF), k1, 1, 1) + jnp.concatenate(
                    [_dg(q0.astype(BF), k0, 1, 1), _dg(q2.astype(BF), k2, 1, 1)], axis=0)
                return sc

            def sm(sc):
                sc = jnp.where(mask, sc * scale, -1e9)
                e = jnp.exp(sc - jnp.max(sc, axis=-1, keepdims=True))
                pr = e * (1.0 / jnp.sum(e, axis=-1, keepdims=True))
                return pr

            def pv(pr, v):
                v0, v1, v2 = v
                om = _dot(pr.astype(BF), v1)
                o = jnp.concatenate([_dot(pr[:L].astype(BF), v0), jnp.where(lo, om[:L], om[L:]),
                                     _dot(pr[L:].astype(BF), v2)], axis=1)
                return o.astype(BF)

            acc = None
            cur = proj(0)
            for g in range(ng):
                nxt = proj(g + 1) if g + 1 < ng else None
                scs = [qk(cur[0][3 * j:3 * j + 3], cur[1][3 * j:3 * j + 3]) for j in range(G)]
                vv = _tiles(_dot(h, wv[:, g * W:(g + 1) * W]).astype(BF))
                prs = [sm(t) for t in scs]
                o = jnp.concatenate([pv(prs[j], vv[3 * j:3 * j + 3]) for j in range(G)], axis=1)
                d = _dot(o, wob[g * W:(g + 1) * W, :])
                acc = d if acc is None else acc + d
                cur = nxt
            xs[r, :] = xr + acc[:seg]
            return acc[seg:seg + M]

        lax.fori_loop(0, S // seg, step, mem_ref[...].astype(F32))

    def layers(i, c):
        layer_a()

        @pl.when(i == 0)
        def _():
            for cp in cps:
                cp.wait()

        layer_b()
        return c

    lax.fori_loop(0, 2, layers, 0)
    o_ref[...] = xs[...].astype(o_ref.dtype)


def pallas_interleave_layers__linear_kernel_hedgehog__memory_aug_recurrent_mem_tr__prompt_kernel(
        A_x, A_wqkv, A_w_phi, A_wo, B_x, B_mem0, B_Wq, B_Wk, B_Wv, B_Wo, B_seg_len=32):
    _, S, D = A_x.shape
    seg = B_seg_len if isinstance(B_seg_len, int) else 32
    HE = B_Wq.shape[1] * B_Wq.shape[2]
    vm = pl.BlockSpec(memory_space=pltpu.VMEM)
    hb = pl.BlockSpec(memory_space=pl.ANY)
    out = pl.pallas_call(
        functools.partial(_kernel, seg),
        in_specs=[vm] * 5 + [hb] * 4,
        out_specs=vm,
        out_shape=jax.ShapeDtypeStruct((S, D), A_x.dtype),
        scratch_shapes=[pltpu.VMEM((S, D), F32), pltpu.VMEM((D, 2 * D), BF), pltpu.VMEM((S, 2 * D), BF),
                        pltpu.VMEM((D, HE), BF), pltpu.VMEM((D, HE), BF), pltpu.VMEM((D, HE), BF),
                        pltpu.VMEM((HE, D), BF), pltpu.SemaphoreType.DMA((4,))],
        compiler_params=pltpu.CompilerParams(vmem_limit_bytes=110 * 1024 * 1024),
    )(A_x.reshape(S, D), A_wqkv, A_w_phi.reshape(D, D // HA), A_wo, B_mem0.reshape(-1, D),
      B_Wq.reshape(D, HE), B_Wk.reshape(D, HE), B_Wv.reshape(D, HE), B_Wo.reshape(HE, D))
    return out.reshape(1, S, D)
```

```python
import functools
import jax
import jax.numpy as jnp
from jax import lax
import jax.experimental.pallas as pl
import jax.experimental.pallas.tpu as pltpu

F32, BF = jnp.float32, jnp.bfloat16
HA = 32
G = 16
CH = 512


def _dot(a, b):
    return jnp.dot(a, b, preferred_element_type=F32)


def _dg(a, b, ca, cb):
    return lax.dot_general(a, b, (((ca,), (cb,)), ((), ())), preferred_element_type=F32)


def _ln(x):
    m = jnp.mean(x, axis=-1, keepdims=True)
    d = x - m
    v = jnp.mean(d * d, axis=-1, keepdims=True)
    return d * lax.rsqrt(v + 1e-5)


def _iota(shape, ax):
    return lax.broadcasted_iota(jnp.int32, shape, ax)


def _tiles(a):
    return [a[:, i * 128:(i + 1) * 128] for i in range(a.shape[1] // 128)]


def _allred(ts, op):
    r = functools.reduce(op, ts)
    r = op(r, pltpu.roll(r, 64, 1))
    return op(r, pltpu.roll(r, 32, 1))


def _phi(p):
    ts = _tiles(p)
    mx = _allred(ts, jnp.maximum)
    mn = _allred(ts, jnp.minimum)
    out = []
    for e in ([jnp.exp(t - mx) for t in ts], [jnp.exp(mn - t) for t in ts]):
        inv = 1.0 / _allred(e, jnp.add)
        out += [t * inv for t in e]
    return out


def _kernel(seg, x_ref, wqkv_ref, wphi_ref, wo_ref, mem_ref, wq_h, wk_h, wv_h, wob_h,
            o_ref, xs, wqk, phiq, wq, wk, wv, wob, sem):
    S, D = xs.shape
    M = mem_ref.shape[0]
    dh = D // HA
    L = seg + 2 * M
    E = 192
    cps = [pltpu.make_async_copy(s, d, sem.at[i]) for i, (s, d) in
           enumerate(((wq_h, wq), (wk_h, wk), (wv_h, wv), (wob_h, wob)))]
    for c in cps:
        c.start()

    rep = (_iota((dh, D), 0) == _iota((dh, D), 1) // HA).astype(BF)
    bd = _dot(wphi_ref[...], rep)
    bd = jnp.where(_iota((D, D), 0) // dh == _iota((D, D), 1) % HA, bd, 0.0).astype(BF)
    wqk[:, :D] = _dot(wqkv_ref[:, :D], bd).astype(BF)
    wqk[:, D:] = _dot(wqkv_ref[:, D:2 * D], bd).astype(BF)
    xs[...] = x_ref[...].astype(F32)

    def layer_a():
        def p1(i, c):
            kvt, z = c
            r = pl.ds(pl.multiple_of(i * CH, CH), CH)
            h = _ln(xs[r, :]).astype(BF)
            phiq[r, :] = jnp.concatenate(_phi(_dot(h, wqk[:, :D])), axis=1).astype(BF)
            pk = jnp.concatenate(_phi(_dot(h, wqk[:, D:])), axis=1)
            v = _dot(h, wqkv_ref[:, 2 * D:]).astype(BF)
            return kvt + _dg(v, pk.astype(BF), 0, 0), z + jnp.sum(pk, axis=0, keepdims=True)

        kvt, z = lax.fori_loop(0, S // CH, p1, (jnp.zeros((D, 2 * D), F32), jnp.zeros((1, 2 * D), F32)))
        kvt = jnp.where(_iota((D, 2 * D), 0) // dh == _iota((D, 2 * D), 1) % HA, kvt, 0.0).astype(BF)
        g = _dg(kvt, wo_ref[...], 0, 0).astype(BF)

        def p2(i, c):
            r = pl.ds(pl.multiple_of(i * CH, CH), CH)
            ts = _tiles(phiq[r, :].astype(F32))
            inv = 1.0 / (_allred([t * zt for t, zt in zip(ts, _tiles(z))], jnp.add) + 1e-6)
            xs[r, :] += _dot(jnp.concatenate([t * inv for t in ts], axis=1).astype(BF), g)
            return c

        lax.fori_loop(0, S // CH, p2, 0)

    def layer_b():
        scale = E ** -0.5
        Q = seg + M
        qi = _iota((2 * Q, L), 0) % Q
        ki = _iota((2 * Q, L), 1)
        mask = (ki < seg + M) & ((qi >= seg) | (ki >= seg) | (qi >= ki))
        lo = _iota((Q, 128), 1) < 64

        def step(s, mem):
            r = pl.ds(pl.multiple_of(s * seg, seg), seg)
            xr = xs[r, :]
            h = jnp.concatenate([_ln(xr), mem], axis=0).astype(BF).astype(F32)

            def pad(h, w):
                t = _dot(h, w)
                return jnp.concatenate([t, jnp.zeros((M, t.shape[1]), F32)], axis=0)

            W = G * 2 * E
            ng = wq.shape[1] // W

            def proj(g):
                c = slice(g * W, (g + 1) * W)
                return (_tiles(_dot(h, wq[:, c])), _tiles(pad(h, wk[:, c]).astype(BF)),
                        None)

            def qk(q, k):
                q0, q1, q2 = q
                k0, k1, k2 = k
                qm = jnp.concatenate([jnp.where(lo, q1, 0.0), jnp.where(lo, 0.0, q1)], axis=0)
                sc = _dg(qm, k1, 1, 1) + jnp.concatenate(
                    [_dg(q0, k0, 1, 1), _dg(q2, k2, 1, 1)], axis=0)
                return sc

            def sm(sc):
                sc = jnp.where(mask, sc * scale, -1e9)
                e = jnp.exp(sc - jnp.max(sc, axis=-1, keepdims=True))
                pr = e * (1.0 / jnp.sum(e, axis=-1, keepdims=True))
                return pr

            def pv(pr, v):
                v0, v1, v2 = v
                om = _dot(pr, v1)
                o = jnp.concatenate([_dot(pr[:Q], v0), jnp.where(lo, om[:Q], om[Q:]),
                                     _dot(pr[Q:], v2)], axis=1)
                return o

            acc = None
            cur = proj(0)
            for g in range(ng):
                nxt = proj(g + 1) if g + 1 < ng else None
                scs = [qk(cur[0][3 * j:3 * j + 3], cur[1][3 * j:3 * j + 3]) for j in range(G)]
                vv = _tiles(pad(h, wv[:, g * W:(g + 1) * W]).astype(BF))
                prs = [sm(t) for t in scs]
                o = jnp.concatenate([pv(prs[j], vv[3 * j:3 * j + 3]) for j in range(G)], axis=1)
                d = _dot(o, wob[g * W:(g + 1) * W, :])
                acc = d if acc is None else acc + d
                cur = nxt
            xs[r, :] = xr + acc[:seg]
            return acc[seg:seg + M]

        lax.fori_loop(0, S // seg, step, mem_ref[...].astype(F32))

    def layers(i, c):
        layer_a()

        @pl.when(i == 0)
        def _():
            for cp in cps:
                cp.wait()

        layer_b()
        return c

    lax.fori_loop(0, 2, layers, 0)
    o_ref[...] = xs[...].astype(o_ref.dtype)


def pallas_interleave_layers__linear_kernel_hedgehog__memory_aug_recurrent_mem_tr__prompt_kernel(
        A_x, A_wqkv, A_w_phi, A_wo, B_x, B_mem0, B_Wq, B_Wk, B_Wv, B_Wo, B_seg_len=32):
    _, S, D = A_x.shape
    seg = B_seg_len if isinstance(B_seg_len, int) else 32
    HE = B_Wq.shape[1] * B_Wq.shape[2]
    vm = pl.BlockSpec(memory_space=pltpu.VMEM)
    hb = pl.BlockSpec(memory_space=pl.ANY)
    out = pl.pallas_call(
        functools.partial(_kernel, seg),
        in_specs=[vm] * 5 + [hb] * 4,
        out_specs=vm,
        out_shape=jax.ShapeDtypeStruct((S, D), A_x.dtype),
        scratch_shapes=[pltpu.VMEM((S, D), F32), pltpu.VMEM((D, 2 * D), BF), pltpu.VMEM((S, 2 * D), BF),
                        pltpu.VMEM((D, HE), BF), pltpu.VMEM((D, HE), BF), pltpu.VMEM((D, HE), BF),
                        pltpu.VMEM((HE, D), BF), pltpu.SemaphoreType.DMA((4,))],
        compiler_params=pltpu.CompilerParams(vmem_limit_bytes=110 * 1024 * 1024),
    )(A_x.reshape(S, D), A_wqkv, A_w_phi.reshape(D, D // HA), A_wo, B_mem0.reshape(-1, D),
      B_Wq.reshape(D, HE), B_Wk.reshape(D, HE), B_Wv.reshape(D, HE), B_Wo.reshape(HE, D))
    return out.reshape(1, S, D)
```
